```python
import os as _os
_os.environ.setdefault("JAX_PLATFORMS", "cpu")
import jax
import jax.numpy as jnp

def _softmax(x, axis=-1):
    return jax.nn.softmax(x, axis=axis)
def _gelu(x):
    return jax.nn.gelu(x, approximate=True)
def _silu(x):
    return jax.nn.silu(x)
def _sigmoid(x):
    return jax.nn.sigmoid(x)
def _layernorm(x, axis=-1, eps=1e-5):
    m = jnp.mean(x, axis=axis, keepdims=True)
    v = jnp.var(x, axis=axis, keepdims=True)
    return (x - m) / jnp.sqrt(v + eps)
def _scatter_add(tgt, idx, src, axis=0):
    return tgt.at[idx].add(src)
def _segment_sum(src, seg, n):
    return jax.ops.segment_sum(src, seg, n)
class _Rng:
    def __init__(self, key):
        self._k = key
    def _next(self):
        self._k, sub = jax.random.split(self._k)
        return sub
    def normal(self, shape):
        return jax.random.normal(self._next(), shape, dtype=jnp.bfloat16)
    def randint(self, lo, hi, shape):
        return jax.random.randint(self._next(), shape, lo, hi, dtype=jnp.int32)
    def uniform(self, shape, lo=0.0, hi=1.0):
        return jax.random.uniform(self._next(), shape, jnp.bfloat16, lo, hi)
    def permutation(self, n):
        return jax.random.permutation(self._next(), n)


kernel_name = 'standalone__detection_seg_fpn_lateral__vision'

def setup_inputs():
    _rng = _Rng(jax.random.key(int.from_bytes(__import__("os").urandom(4), "little")))
    _w = (lambda a: (lambda t: t.astype(jnp.bfloat16) if jnp.issubdtype(t.dtype, jnp.floating) else t)(jnp.asarray(a)))
    H = W = (256 // 2) * 2
    C = 384
    k = 1
    return {
        "c_fine": _w((lambda *s: _rng.normal(s) * 0.05)(1, H, W, C)),
        "p_coarse": _w((lambda *s: _rng.normal(s) * 0.05)(1, H // 2, W // 2, C)),
        "w_lat": _w((lambda *s: _rng.normal(s) * 0.05)(C, C)),
        "w_out": _w((lambda *s: _rng.normal(s) * 0.05)(k, k, C, C)),
    }

def reference(c_fine, p_coarse, w_lat, w_out):
    B, H, W, C = c_fine.shape
    k = 1
    lat = jnp.einsum("bhwc,cd->bhwd", c_fine, w_lat)
    up = jnp.repeat(jnp.repeat(p_coarse, 2, axis=1), 2, axis=2)
    m = lat + up
    pad = k // 2
    mp = jnp.pad(m, ((0, 0), (pad, pad), (pad, pad), (0, 0)))
    o = None
    for di in range(k):
        for dj in range(k):
            t = jnp.einsum("bhwc,cd->bhwd", mp[:, di:di + H, dj:dj + W, :], w_out[di, dj])
            o = t if o is None else o + t
    return o
```

```python
import jax
import jax.numpy as jnp
from jax import lax
import jax.experimental.pallas as pl
import jax.experimental.pallas.tpu as pltpu

_S = 8
_R = 32
_U = 4
_G0 = 18
_W0 = 64
_WPER = 16


@jax.jit
def pallas_standalone__detection_seg_fpn_lateral__vision_kernel(
    c_fine: jax.Array,
    p_coarse: jax.Array,
    w_lat: jax.Array,
    w_out: jax.Array,
):
    B, H, W, C = c_fine.shape
    assert B == 1 and w_out.shape[:2] == (1, 1)
    S, R, U = _S, _R, _U
    W2 = W // 2
    T = (H // 2) // S
    nj = (2 * W) // R
    nw = T * nj
    gps = S // U
    G = T * gps
    nl = C // 128
    dt = c_fine.dtype

    def kern(c_hbm, p_hbm, wl_hbm, wo_hbm, o_hbm, cbuf, pbuf, obuf, wl, wo, wc, up_ref, sem):
        def rd_c(t):
            sl = pl.ds(t * 2 * W, 2 * W)
            return pltpu.make_async_copy(c_hbm.at[:, sl], cbuf.at[:, sl], sem.at[t])

        def rd_p(t):
            sl = pl.ds(t * W2, W2)
            return pltpu.make_async_copy(p_hbm.at[:, sl], pbuf.at[:, sl], sem.at[t])

        def wr(d):
            sl = pl.ds(pl.multiple_of(d * R, R), R)
            return pltpu.make_async_copy(obuf.at[:, sl], o_hbm.at[:, sl], sem.at[T + 1])

        cwl = pltpu.make_async_copy(wl_hbm, wl, sem.at[T])
        cwo = pltpu.make_async_copy(wo_hbm, wo, sem.at[T])
        cwo.start()
        cwl.start()
        for t in range(T):
            rd_p(t).start()
            rd_c(t).start()
        cwo.wait()
        cwl.wait()
        wc[...] = jnp.dot(wl[...], wo[...], preferred_element_type=jnp.float32).astype(dt)

        def compute_group(g):
            t = g // gps
            for u in range(U):
                s = (g % gps) * U + u
                poff = pl.multiple_of(t * W2, W2)
                q = jnp.dot(pbuf[s, pl.ds(poff, W2), :], wo[...],
                            preferred_element_type=jnp.float32)
                for j in range(nl):
                    qj = q[:, j * 128:(j + 1) * 128]
                    up_ref[u, j, pl.ds(0, W2, stride=2), :] = qj
                    up_ref[u, j, pl.ds(1, W2, stride=2), :] = qj
                up = jnp.concatenate([up_ref[u, j] for j in range(nl)], axis=1)
                for rr in range(2):
                    off = pl.multiple_of(t * 2 * W + rr * W, W)
                    acc = jnp.dot(cbuf[s, pl.ds(off, W), :], wc[...],
                                  preferred_element_type=jnp.float32)
                    obuf[s, pl.ds(off, W), :] = (acc + up).astype(dt)

        def write_range(lo, hi):
            def body(d, carry):
                wr(d).start()
                return carry
            lax.fori_loop(lo, hi, body, 0)

        def wait_reads(t, carry):
            rd_p(t).wait()
            rd_c(t).wait()
            return carry

        def phase1(g, carry):
            @pl.when(g % gps == 0)
            def _():
                wait_reads(g // gps, 0)
            compute_group(g)
            return carry

        lax.fori_loop(0, _G0, phase1, 0)
        lax.fori_loop((_G0 + gps - 1) // gps, T, wait_reads, 0)
        w0 = min(_W0, (_G0 // gps) * nj)
        write_range(0, w0)

        def phase2(g, issued):
            compute_group(g)
            hi = jnp.minimum(issued + _WPER, ((g + 1) // gps) * nj)
            write_range(issued, hi)
            return hi

        issued = lax.fori_loop(_G0, G, phase2, w0)
        write_range(issued, nw)
        pltpu.make_async_copy(obuf, o_hbm, sem.at[T + 1]).wait()

    c = c_fine.reshape(S, T * 2 * W, C)
    p = p_coarse.reshape(S, T * W2, C)
    out = pl.pallas_call(
        kern,
        in_specs=[pl.BlockSpec(memory_space=pl.ANY)] * 4,
        out_specs=pl.BlockSpec(memory_space=pl.ANY),
        out_shape=jax.ShapeDtypeStruct((S, T * 2 * W, C), dt),
        scratch_shapes=[
            pltpu.VMEM((S, T * 2 * W, C), dt),
            pltpu.VMEM((S, T * W2, C), dt),
            pltpu.VMEM((S, T * 2 * W, C), dt),
            pltpu.VMEM((C, C), dt),
            pltpu.VMEM((C, C), dt),
            pltpu.VMEM((C, C), dt),
            pltpu.VMEM((U, nl, W, 128), jnp.float32),
            pltpu.SemaphoreType.DMA((T + 2,)),
        ],
        compiler_params=pltpu.CompilerParams(vmem_limit_bytes=124 * 1024 * 1024),
    )(c, p, w_lat, w_out.reshape(C, C))
    return out.reshape(B, H, W, C)
```

```python
import jax
import jax.numpy as jnp
from jax import lax
import jax.experimental.pallas as pl
import jax.experimental.pallas.tpu as pltpu

_A = 2
_RR = 16
_RW = 32
_NC = (7, 6, 7, 6)
_NP = (2, 2, 2, 1)
_G1 = 17
_EC = 8
_QA = 7
_NLO = 3
_W0 = 64
_WPER = 16
_HI, _LO = 0, 1


@jax.jit
def pallas_standalone__detection_seg_fpn_lateral__vision_kernel(
    c_fine: jax.Array,
    p_coarse: jax.Array,
    w_lat: jax.Array,
    w_out: jax.Array,
):
    B, H, W, C = c_fine.shape
    assert B == 1 and w_out.shape[:2] == (1, 1)
    dt = c_fine.dtype
    A, RR, RW = _A, _RR, _RW
    W2 = W // 2
    nl = C // 128
    nstep = (H // 2) // 8
    T = nstep // A
    LC, LP = T * 2 * W, T * W2
    cps, pps = (2 * W) // RR, W2 // RR
    NC, NP = nstep * cps, nstep * pps
    nj = (2 * W) // RW
    nw = nstep * nj
    NG = 2 * nstep
    SEM_W, SEM_O, SEM_T = 2 * NG, 2 * NG + 1, 2 * NG + 2
    c0 = NC - _EC - _G1 * sum(_NC)
    p0 = NP - _G1 * sum(_NP)
    gt = _G1 + 1
    w0 = min(_W0, (gt // 2) * nj)
    assert c0 >= 4 * _QA and p0 >= _QA and gt <= NG - 2 and 0 < _EC < cps
    for g in range(_G1):
        assert c0 + g * sum(_NC) >= (g // 2 + 1) * cps
        assert p0 + g * sum(_NP) >= (g // 2 + 1) * pps

    def kern(c_hbm, p_hbm, wl_hbm, wo_hbm, o_hbm, cbuf, pbuf, obuf, wl, wo, wc, up_ref, sem):
        def loop(lo, hi, f):
            def body(x, carry):
                f(x)
                return carry
            lax.fori_loop(lo, hi, body, 0)

        def start_c(i, tail=False, prio=(_HI, _LO)):
            a = i // (T * cps)
            sl = pl.ds(pl.multiple_of((i % (T * cps)) * RR, RR), RR)
            for h in range(2):
                s = SEM_T if tail else 2 * (i // cps) + h
                pltpu.make_async_copy(c_hbm.at[a, h, :, sl], cbuf.at[a, h, :, sl],
                                      sem.at[s]).start(priority=prio[h])

        def start_p(i, prio=(_HI, _LO)):
            a = i // (T * pps)
            sl = pl.ds(pl.multiple_of((i % (T * pps)) * RR, RR), RR)
            for h in range(2):
                pltpu.make_async_copy(p_hbm.at[a, h, :, sl], pbuf.at[a, h, :, sl],
                                      sem.at[NG + 2 * (i // pps) + h]).start(priority=prio[h])

        def start_bundle(x, prio=(_HI, _LO)):
            start_p(x, prio)
            for i in range(4):
                start_c(4 * x + i, prio=prio)

        def wait_group(g, ncp=cps):
            k, h = g // 2, g % 2
            a, t = k // T, k % T
            sl = pl.ds(pl.multiple_of(t * 2 * W, RR), ncp * RR)
            pltpu.make_async_copy(c_hbm.at[a, h, :, sl], cbuf.at[a, h, :, sl], sem.at[g]).wait()
            sl = pl.ds(pl.multiple_of(t * W2, RR), W2)
            pltpu.make_async_copy(p_hbm.at[a, h, :, sl], pbuf.at[a, h, :, sl], sem.at[NG + g]).wait()

        def start_w(d):
            a = d // (T * nj)
            sl = pl.ds(pl.multiple_of((d % (T * nj)) * RW, RW), RW)
            pltpu.make_async_copy(obuf.at[a, :, sl], o_hbm.at[a, :, sl], sem.at[SEM_O]).start()

        def compute_unit(g, u):
            k, h = g // 2, g % 2
            a, t = k // T, k % T
            q = jnp.dot(pbuf[a, h, u, pl.ds(pl.multiple_of(t * W2, W2), W2), :], wo[...],
                        preferred_element_type=jnp.float32)
            for j in range(nl):
                qj = q[:, j * 128:(j + 1) * 128]
                up_ref[u, j, pl.ds(0, W2, stride=2), :] = qj
                up_ref[u, j, pl.ds(1, W2, stride=2), :] = qj
            up = jnp.concatenate([up_ref[u, j] for j in range(nl)], axis=1)
            for rr in range(2):
                sl = pl.ds(pl.multiple_of(t * 2 * W + rr * W, W), W)
                acc = jnp.dot(cbuf[a, h, u, sl, :], wc[...], preferred_element_type=jnp.float32)
                obuf[a, 4 * h + u, sl, :] = (acc + up).astype(dt)

        cwl = pltpu.make_async_copy(wl_hbm, wl, sem.at[SEM_W])
        cwo = pltpu.make_async_copy(wo_hbm, wo, sem.at[SEM_W])
        cwo.start(priority=_HI)
        cwl.start(priority=_HI)
        loop(0, _NLO, lambda x: start_bundle(x, (_LO, _LO)))
        loop(_NLO, _QA, start_bundle)
        cwo.wait()
        cwl.wait()
        wc[...] = jnp.dot(wl[...], wo[...], preferred_element_type=jnp.float32).astype(dt)
        loop(_QA, p0, start_p)
        loop(4 * _QA, c0, start_c)

        def phase1(g):
            wait_group(g)
            ic = c0 + g * sum(_NC)
            ip = p0 + g * sum(_NP)
            for u in range(4):
                compute_unit(g, u)
                for i in range(_NC[u]):
                    if i < _NP[u]:
                        start_p(ip)
                        ip += 1
                    start_c(ic)
                    ic += 1

        loop(0, _G1, phase1)
        loop(NC - _EC, NC, lambda i: start_c(i, tail=True))

        def phase2(g, issued):
            @pl.when(g < gt)
            def _():
                wait_group(g)

            @pl.when(g == gt)
            def _():
                loop(gt, NG - 2, wait_group)
                wait_group(NG - 2, cps - _EC)
                wait_group(NG - 1, cps - _EC)
                loop(0, w0, start_w)
                sl = pl.ds(LC - _EC * RR, _EC * RR)
                pltpu.make_async_copy(c_hbm.at[A - 1, :, :, sl], cbuf.at[A - 1, :, :, sl],
                                      sem.at[SEM_T]).wait()

            for u in range(4):
                compute_unit(g, u)
            hi = jnp.minimum(issued + _WPER, ((g + 1) // 2) * nj)
            hi = jnp.where(g < gt, issued, hi)
            loop(issued, hi, start_w)
            return hi

        issued = lax.fori_loop(_G1, NG, phase2, w0)
        loop(issued, nw, start_w)
        pltpu.make_async_copy(obuf, o_hbm, sem.at[SEM_O]).wait()

    out = pl.pallas_call(
        kern,
        in_specs=[pl.BlockSpec(memory_space=pl.ANY)] * 4,
        out_specs=pl.BlockSpec(memory_space=pl.ANY),
        out_shape=jax.ShapeDtypeStruct((A, 8, LC, C), dt),
        scratch_shapes=[
            pltpu.VMEM((A, 2, 4, LC, C), dt),
            pltpu.VMEM((A, 2, 4, LP, C), dt),
            pltpu.VMEM((A, 8, LC, C), dt),
            pltpu.VMEM((C, C), dt),
            pltpu.VMEM((C, C), dt),
            pltpu.VMEM((C, C), dt),
            pltpu.VMEM((4, nl, W, 128), jnp.float32),
            pltpu.SemaphoreType.DMA((2 * NG + 3,)),
        ],
        compiler_params=pltpu.CompilerParams(
            vmem_limit_bytes=124 * 1024 * 1024,
            disable_bounds_checks=True,
            disable_semaphore_checks=True,
        ),
    )(c_fine.reshape(A, 2, 4, LC, C), p_coarse.reshape(A, 2, 4, LP, C),
      w_lat, w_out.reshape(C, C))
    return out.reshape(B, H, W, C)
```

```python
import jax
import jax.numpy as jnp
from jax import lax
import jax.experimental.pallas as pl
import jax.experimental.pallas.tpu as pltpu

_A = 2
_RR = 16
_RW = 32
_NC = (7, 7, 7, 6)
_NP = (2, 2, 2, 1)
_G1 = 17
_EC = 8
_QA = 9
_NLO = 3
_W0 = 64
_WPER = 16
_HI, _LO = 0, 1


def _divmod(x, n):
    assert n > 0 and n & (n - 1) == 0
    return x >> (n.bit_length() - 1), x & (n - 1)


@jax.jit
def pallas_standalone__detection_seg_fpn_lateral__vision_kernel(
    c_fine: jax.Array,
    p_coarse: jax.Array,
    w_lat: jax.Array,
    w_out: jax.Array,
):
    B, H, W, C = c_fine.shape
    assert B == 1 and w_out.shape[:2] == (1, 1)
    dt = c_fine.dtype
    A, RR, RW = _A, _RR, _RW
    W2 = W // 2
    nl = C // 128
    nstep = (H // 2) // 8
    T = nstep // A
    LC, LP = T * 2 * W, T * W2
    cps, pps = (2 * W) // RR, W2 // RR
    NC, NP = nstep * cps, nstep * pps
    nj = (2 * W) // RW
    nw = nstep * nj
    NG = 2 * nstep
    SEM_W, SEM_O, SEM_T = 2 * NG, 2 * NG + 1, 2 * NG + 2
    c0 = NC - _EC - _G1 * sum(_NC)
    p0 = NP - _G1 * sum(_NP)
    gt = _G1 + 1
    w0 = min(_W0, (gt // 2) * nj)
    assert c0 >= 4 * _QA and p0 >= _QA and gt <= NG - 2 and 0 < _EC < cps
    for g in range(_G1):
        assert c0 + g * sum(_NC) >= (g // 2 + 1) * cps
        assert p0 + g * sum(_NP) >= (g // 2 + 1) * pps

    def kern(c_hbm, p_hbm, wl_hbm, wo_hbm, o_hbm, cbuf, pbuf, obuf, wl, wo, wc, up_ref, sem):
        def loop(lo, hi, f):
            def body(x, carry):
                f(x)
                return carry
            lax.fori_loop(lo, hi, body, 0)

        def start_c(i, tail=False, prio=(_HI, _LO)):
            a, j = _divmod(i, T * cps)
            sl = pl.ds(pl.multiple_of(j * RR, RR), RR)
            for h in range(2):
                s = SEM_T if tail else 2 * _divmod(i, cps)[0] + h
                pltpu.make_async_copy(c_hbm.at[a, h, :, sl], cbuf.at[a, h, :, sl],
                                      sem.at[s]).start(priority=prio[h])

        def start_p(i, prio=(_HI, _LO)):
            a, j = _divmod(i, T * pps)
            sl = pl.ds(pl.multiple_of(j * RR, RR), RR)
            for h in range(2):
                s = NG + 2 * _divmod(i, pps)[0] + h
                pltpu.make_async_copy(p_hbm.at[a, h, :, sl], pbuf.at[a, h, :, sl],
                                      sem.at[s]).start(priority=prio[h])

        def start_bundle(x, prio=(_HI, _LO)):
            start_p(x, prio)
            for i in range(4):
                start_c(4 * x + i, prio=prio)

        def wait_group(g, ncp=cps):
            k, h = _divmod(g, 2)
            a, t = _divmod(k, T)
            sl = pl.ds(pl.multiple_of(t * 2 * W, RR), ncp * RR)
            pltpu.make_async_copy(c_hbm.at[a, h, :, sl], cbuf.at[a, h, :, sl], sem.at[g]).wait()
            sl = pl.ds(pl.multiple_of(t * W2, RR), W2)
            pltpu.make_async_copy(p_hbm.at[a, h, :, sl], pbuf.at[a, h, :, sl], sem.at[NG + g]).wait()

        def start_w(d):
            a, j = _divmod(d, T * nj)
            sl = pl.ds(pl.multiple_of(j * RW, RW), RW)
            pltpu.make_async_copy(obuf.at[a, :, sl], o_hbm.at[a, :, sl], sem.at[SEM_O]).start()

        def compute_unit(g, u):
            k, h = _divmod(g, 2)
            a, t = _divmod(k, T)
            q = jnp.dot(pbuf[a, h, u, pl.ds(pl.multiple_of(t * W2, W2), W2), :], wo[...],
                        preferred_element_type=jnp.float32)
            for j in range(nl):
                qj = q[:, j * 128:(j + 1) * 128]
                up_ref[u, j, pl.ds(0, W2, stride=2), :] = qj
                up_ref[u, j, pl.ds(1, W2, stride=2), :] = qj
            up = jnp.concatenate([up_ref[u, j, pl.ds(0, W), :] for j in range(nl)], axis=1)
            for rr in range(2):
                sl = pl.ds(pl.multiple_of(t * 2 * W + rr * W, W), W)
                acc = jnp.dot(cbuf[a, h, u, sl, :], wc[...], preferred_element_type=jnp.float32)
                obuf[a, 4 * h + u, sl, :] = (acc + up).astype(dt)

        cwl = pltpu.make_async_copy(wl_hbm, wl, sem.at[SEM_W])
        cwo = pltpu.make_async_copy(wo_hbm, wo, sem.at[SEM_W])
        cwo.start(priority=_HI)
        cwl.start(priority=_HI)
        loop(0, _NLO, lambda x: start_bundle(x, (_LO, _LO)))
        loop(_NLO, _QA, start_bundle)
        up_ref[...] = jnp.zeros(up_ref.shape, up_ref.dtype)
        cwo.wait()
        cwl.wait()
        wc[...] = jnp.dot(wl[...], wo[...], preferred_element_type=jnp.float32).astype(dt)
        loop(_QA, p0, start_p)
        loop(4 * _QA, c0, start_c)

        def phase1(g):
            wait_group(g)
            ic = c0 + g * sum(_NC)
            ip = p0 + g * sum(_NP)
            for u in range(4):
                compute_unit(g, u)
                for i in range(_NC[u]):
                    if i < _NP[u]:
                        start_p(ip)
                        ip += 1
                    start_c(ic)
                    ic += 1

        loop(0, _G1, phase1)
        loop(NC - _EC, NC, lambda i: start_c(i, tail=True))

        def phase2(g, issued):
            @pl.when(g < gt)
            def _():
                wait_group(g)

            @pl.when(g == gt)
            def _():
                loop(gt, NG - 2, wait_group)
                wait_group(NG - 2, cps - _EC)
                wait_group(NG - 1, cps - _EC)
                loop(0, w0, start_w)
                sl = pl.ds(LC - _EC * RR, _EC * RR)
                pltpu.make_async_copy(c_hbm.at[A - 1, :, :, sl], cbuf.at[A - 1, :, :, sl],
                                      sem.at[SEM_T]).wait()

            for u in range(4):
                compute_unit(g, u)
            hi = jnp.minimum(issued + _WPER, _divmod(g + 1, 2)[0] * nj)
            hi = jnp.where(g < gt, issued, hi)
            loop(issued, hi, start_w)
            return hi

        issued = lax.fori_loop(_G1, NG, phase2, w0)
        loop(issued, nw, start_w)
        pltpu.make_async_copy(obuf, o_hbm, sem.at[SEM_O]).wait()

    out = pl.pallas_call(
        kern,
        in_specs=[pl.BlockSpec(memory_space=pl.ANY)] * 4,
        out_specs=pl.BlockSpec(memory_space=pl.ANY),
        out_shape=jax.ShapeDtypeStruct((A, 8, LC, C), dt),
        scratch_shapes=[
            pltpu.VMEM((A, 2, 4, LC, C), dt),
            pltpu.VMEM((A, 2, 4, LP, C), dt),
            pltpu.VMEM((A, 8, LC, C), dt),
            pltpu.VMEM((C, C), dt),
            pltpu.VMEM((C, C), dt),
            pltpu.VMEM((C, C), dt),
            pltpu.VMEM((4, nl, W + 8, 128), jnp.float32),
            pltpu.SemaphoreType.DMA((2 * NG + 3,)),
        ],
        compiler_params=pltpu.CompilerParams(
            vmem_limit_bytes=124 * 1024 * 1024,
            disable_bounds_checks=True,
            disable_semaphore_checks=True,
        ),
    )(c_fine.reshape(A, 2, 4, LC, C), p_coarse.reshape(A, 2, 4, LP, C),
      w_lat, w_out.reshape(C, C))
    return out.reshape(B, H, W, C)
```
